```python
import os as _os
_os.environ.setdefault("JAX_PLATFORMS", "cpu")
import jax
import jax.numpy as jnp

def _softmax(x, axis=-1):
    return jax.nn.softmax(x, axis=axis)
def _gelu(x):
    return jax.nn.gelu(x, approximate=True)
def _silu(x):
    return jax.nn.silu(x)
def _sigmoid(x):
    return jax.nn.sigmoid(x)
def _layernorm(x, axis=-1, eps=1e-5):
    m = jnp.mean(x, axis=axis, keepdims=True)
    v = jnp.var(x, axis=axis, keepdims=True)
    return (x - m) / jnp.sqrt(v + eps)
def _scatter_add(tgt, idx, src, axis=0):
    return tgt.at[idx].add(src)
def _segment_sum(src, seg, n):
    return jax.ops.segment_sum(src, seg, n)
class _Rng:
    def __init__(self, key):
        self._k = key
    def _next(self):
        self._k, sub = jax.random.split(self._k)
        return sub
    def normal(self, shape):
        return jax.random.normal(self._next(), shape, dtype=jnp.bfloat16)
    def randint(self, lo, hi, shape):
        return jax.random.randint(self._next(), shape, lo, hi, dtype=jnp.int32)
    def uniform(self, shape, lo=0.0, hi=1.0):
        return jax.random.uniform(self._next(), shape, jnp.bfloat16, lo, hi)
    def permutation(self, n):
        return jax.random.permutation(self._next(), n)


kernel_name = 'standalone__softmax_full_bidir__sampling'

def setup_inputs():
    _rng = _Rng(jax.random.key(int.from_bytes(__import__("os").urandom(4), "little")))
    _w = (lambda a: (lambda t: t.astype(jnp.bfloat16) if jnp.issubdtype(t.dtype, jnp.floating) else t)(jnp.asarray(a)))
    B, H, Sq, Skv, Dh = 8, 32, 1, 4096, 192
    return {
        "q": _w((lambda *s: _rng.normal(s) * 0.4)(B, H, Sq, Dh)),
        "k": _w((lambda *s: _rng.normal(s) * 0.4)(B, H, Skv, Dh)),
        "v": _w((lambda *s: _rng.normal(s) * 0.05)(B, H, Skv, Dh)),
    }

def reference(q, k, v):
    scale = q.shape[-1] ** -0.5
    scores = jnp.einsum('bhqd,bhkd->bhqk', q, k) * scale
    attn = _softmax(scores, axis=-1)
    return jnp.einsum('bhqk,bhkd->bhqd', attn, v)
```

```python
import jax
import jax.numpy as jnp
from jax import lax
import jax.experimental.pallas as pl
import jax.experimental.pallas.tpu as pltpu

_NBUF = 3


def _copy_schedule(dh, skv):
    rows, cols = 8, min(2048, skv)
    piece = lambda op: [(op, r, c, rows, cols) for r in range(0, dh, rows) for c in range(0, skv, cols)]
    k, v = piece(0), piece(1)
    half = len(k) // 2
    order = [x for t in zip(k[:half], v[:half], k[half:], v[half:]) for x in t]
    return [x + (i % 2,) for i, x in enumerate(order)]


@jax.jit
def pallas_standalone__softmax_full_bidir__sampling_kernel(
    q: jax.Array,
    k: jax.Array,
    v: jax.Array,
):
    batch, heads, sq, dh = q.shape
    skv = k.shape[2]
    assert sq == 1
    nh = batch * heads
    scale = dh ** -0.5
    schedule = _copy_schedule(dh, skv)

    def kernel_function(q_hbm, k_hbm, v_hbm, o_hbm, qbuf, qf32, of32, obuf, kbuf, vbuf, sem, iosem):
        def start(h, slot):
            srcs = (k_hbm.at[h], v_hbm.at[h])
            dsts = (kbuf.at[slot], vbuf.at[slot])
            for op, r, c, nr, nc, thread in schedule:
                pltpu.make_async_copy(
                    srcs[op].at[pl.ds(r, nr), pl.ds(c, nc)],
                    dsts[op].at[pl.ds(r, nr), pl.ds(c, nc)],
                    sem.at[slot],
                ).start(priority=thread)

        def wait(slot):
            pltpu.make_async_copy(kbuf.at[slot], kbuf.at[slot], sem.at[slot]).wait()
            pltpu.make_async_copy(vbuf.at[slot], vbuf.at[slot], sem.at[slot]).wait()

        q_copy = pltpu.make_async_copy(q_hbm, qbuf, iosem.at[0])
        q_copy.start()
        lax.fori_loop(0, _NBUF - 1, lambda i, _: start(i, i), None)
        q_copy.wait()
        qf32[...] = qbuf[...].astype(jnp.float32)

        def body(h, slot):
            free_slot = jnp.where(slot == 0, _NBUF - 1, slot - 1)

            @pl.when(h + _NBUF - 1 < nh)
            def _():
                start(h + _NBUF - 1, free_slot)

            wait(slot)
            q8 = jnp.broadcast_to(qf32[pl.ds(h, 1), :], (8, dh)).astype(kbuf.dtype)
            s = jnp.dot(q8, kbuf[slot], preferred_element_type=jnp.float32) * scale
            e = jnp.exp(s - jnp.max(s, axis=-1, keepdims=True))
            denom = jnp.sum(e, axis=-1, keepdims=True)
            o = lax.dot_general(
                e.astype(vbuf.dtype), vbuf[slot], (((1,), (1,)), ((), ())),
                preferred_element_type=jnp.float32,
            )
            of32[pl.ds(h, 1), :] = (o / denom)[0:1]
            return jnp.where(slot == _NBUF - 1, 0, slot + 1)

        lax.fori_loop(0, nh, body, jnp.int32(0))
        obuf[...] = of32[...].astype(obuf.dtype)
        o_copy = pltpu.make_async_copy(obuf, o_hbm, iosem.at[1])
        o_copy.start()
        o_copy.wait()

    kt = jnp.swapaxes(k, 2, 3).reshape(nh, dh, skv)
    vt = jnp.swapaxes(v, 2, 3).reshape(nh, dh, skv)
    hbm = pl.BlockSpec(memory_space=pl.ANY)
    out = pl.pallas_call(
        kernel_function,
        in_specs=[hbm, hbm, hbm],
        out_specs=hbm,
        out_shape=jax.ShapeDtypeStruct((nh, dh), q.dtype),
        scratch_shapes=[
            pltpu.VMEM((nh, dh), q.dtype),
            pltpu.VMEM((nh, dh), jnp.float32),
            pltpu.VMEM((nh, dh), jnp.float32),
            pltpu.VMEM((nh, dh), q.dtype),
            pltpu.VMEM((_NBUF, dh, skv), k.dtype),
            pltpu.VMEM((_NBUF, dh, skv), v.dtype),
            pltpu.SemaphoreType.DMA((_NBUF,)),
            pltpu.SemaphoreType.DMA((2,)),
        ],
        compiler_params=pltpu.CompilerParams(vmem_limit_bytes=64 * 1024 * 1024),
    )(q.reshape(nh, dh), kt, vt)
    return out.reshape(batch, heads, sq, dh)
```

```python
import jax
import jax.numpy as jnp
from jax import lax
import jax.experimental.pallas as pl
import jax.experimental.pallas.tpu as pltpu

_K, _V = 0, 1
_ROWS = 8
_STREAMS = 4
_SLOTS = _STREAMS + 1
_BACKLOG = 16
_LANES = 128
_LATE_ROWS = 16


def _interleave(*lists):
    out = []
    for i in range(max(map(len, lists))):
        out += [l[i] for l in lists if i < len(l)]
    return out


def _spread(blocks, n):
    size = -(-len(blocks) // n)
    return _interleave(*[blocks[i:i + size] for i in range(0, len(blocks), size)])


@jax.jit
def pallas_standalone__softmax_full_bidir__sampling_kernel(
    q: jax.Array,
    k: jax.Array,
    v: jax.Array,
):
    batch, heads, sq, dh = q.shape
    skv = k.shape[2]
    nh = batch * heads
    assert sq == 1 and dh % (_ROWS * _STREAMS) == 0 and dh > _LANES
    scale = dh ** -0.5
    nblocks = dh // _ROWS
    per_step = nblocks // _STREAMS
    half = skv // 2
    last = nh - 1
    drain_step = nh - _STREAMS
    early = nh - _LATE_ROWS

    def kernel_function(q_hbm, k_hbm, v_hbm, o_hbm, q_in, q_f32, o_f32, o_out,
                        k_buf, v_buf, k_sem, v_sem, misc_sem):
        src, dst, sem = (k_hbm, v_hbm), (k_buf, v_buf), (k_sem, v_sem)

        def block(op, head, slot, idx):
            return op, head, slot, idx, sem[op].at[slot]

        def fetch(thread0, thread1):
            halves = [
                [(thread, *b, col) for b in blocks for col in (0, half)]
                for thread, blocks in enumerate((thread0, thread1))
            ]
            for thread, op, head, slot, idx, done, col in _interleave(*halves):
                window = (pl.ds(idx * _ROWS, _ROWS), pl.ds(col, half))
                pltpu.make_async_copy(
                    src[op].at[(head, *window)], dst[op].at[(slot, *window)], done
                ).start(priority=thread)

        def next_slot(slot):
            return jnp.where(slot == _SLOTS - 1, 0, slot + 1)

        def fetch_step(head, slots):
            fetch(*[
                [block(op, head + j, slots[j], (_STREAMS - 1 - j) * per_step + i)
                 for i in range(per_step) for j in range(_STREAMS)]
                for op in (_K, _V)
            ])

        def wait(ref, done):
            pltpu.make_async_copy(ref, ref, done).wait()

        def softmax_weights(head, slot):
            q8 = jnp.broadcast_to(q_f32[pl.ds(head, 1), :], (8, dh)).astype(k_buf.dtype)
            s = jnp.dot(q8, k_buf[slot], preferred_element_type=jnp.float32) * scale
            e = jnp.exp(s - jnp.max(s, axis=-1, keepdims=True))
            return e.astype(v_buf.dtype), 1.0 / jnp.sum(e, axis=-1, keepdims=True)

        def weighted_sum(e, inv_denom, vt):
            out = lax.dot_general(
                e, vt, (((1,), (1,)), ((), ())), preferred_element_type=jnp.float32
            )
            return (out * inv_denom)[0:1]

        q_copy = pltpu.make_async_copy(q_hbm, q_in, misc_sem.at[0])
        q_copy.start()
        k_fill, v_fill = [
            _interleave(*[
                [block(op, j, j, i) for i in range((_STREAMS - 1 - j) * per_step)]
                for j in range(_STREAMS - 1)
            ])
            for op in (_K, _V)
        ]
        cut = len(k_fill) - _BACKLOG // 2
        fetch([], v_fill[:_BACKLOG])
        fetch(k_fill[:cut], v_fill[_BACKLOG:] + k_fill[cut:])
        fetch_step(0, range(_STREAMS))
        q_copy.wait()
        q_f32[...] = q_in[...].astype(jnp.float32)

        def left(op, j):
            head = drain_step + j
            return [block(op, head, head % _SLOTS, i)
                    for i in range((_STREAMS - j) * per_step, nblocks)]

        tail_sem = misc_sem.at[1]
        k_last, v_last = _spread(left(_K, _STREAMS - 1), 2), left(_V, _STREAMS - 1)
        order = _interleave(*[_spread(left(_K, j), j) for j in range(1, _STREAMS - 1)])
        for j in range(1, _STREAMS - 2):
            order += _spread(left(_V, j), 2)
        order += _interleave(_spread(left(_V, _STREAMS - 2), 2), k_last[:8]) + k_last[8:]
        order += _spread([b for b in v_last if b[3] * _ROWS < _LANES], 2)
        order += _spread([(*b[:4], tail_sem) for b in v_last if b[3] * _ROWS >= _LANES], 2)
        drain0 = order[:_BACKLOG] + order[_BACKLOG:-_BACKLOG:2]
        drain1 = order[_BACKLOG + 1:-_BACKLOG:2] + order[-_BACKLOG:]

        def step(head, slot):
            slots = [next_slot(slot)]
            for _ in range(_STREAMS - 1):
                slots.append(next_slot(slots[-1]))

            @pl.when(head < drain_step)
            def _():
                fetch_step(head + 1, slots)

            @pl.when(head == drain_step)
            def _():
                fetch(drain0[:nblocks], drain1[:nblocks])
                o_out[:early] = o_f32[:early].astype(o_out.dtype)

            @pl.when(head == drain_step + 1)
            def _():
                fetch(drain0[nblocks:], drain1[nblocks:])

            wait(k_buf.at[slot], k_sem.at[slot])
            wait(v_buf.at[slot], v_sem.at[slot])
            e, inv_denom = softmax_weights(head, slot)
            o_f32[pl.ds(head, 1), :] = weighted_sum(e, inv_denom, v_buf[slot])
            return slots[0]

        lax.fori_loop(0, last, step, jnp.int32(0))

        slot = last % _SLOTS
        wait(k_buf.at[slot], k_sem.at[slot])
        e, inv_denom = softmax_weights(last, slot)
        v_lo = v_buf.at[slot, pl.ds(0, _LANES)]
        v_hi = v_buf.at[slot, pl.ds(_LANES, dh - _LANES)]
        wait(v_lo, v_sem.at[slot])
        early_copy = pltpu.make_async_copy(
            o_out.at[pl.ds(0, early)], o_hbm.at[pl.ds(0, early)], misc_sem.at[0]
        )
        early_copy.start()
        o_f32[last:, :_LANES] = weighted_sum(e, inv_denom, v_lo[...])
        wait(v_hi, tail_sem)
        o_f32[last:, _LANES:] = weighted_sum(e, inv_denom, v_hi[...])
        o_out[early:] = o_f32[early:].astype(o_out.dtype)
        late_copy = pltpu.make_async_copy(
            o_out.at[pl.ds(early, _LATE_ROWS)], o_hbm.at[pl.ds(early, _LATE_ROWS)],
            misc_sem.at[2],
        )
        late_copy.start()
        early_copy.wait()
        late_copy.wait()

    kt = jnp.swapaxes(k, 2, 3).reshape(nh, dh, skv)
    vt = jnp.swapaxes(v, 2, 3).reshape(nh, dh, skv)
    hbm = pl.BlockSpec(memory_space=pl.ANY)
    out = pl.pallas_call(
        kernel_function,
        in_specs=[hbm, hbm, hbm],
        out_specs=hbm,
        out_shape=jax.ShapeDtypeStruct((nh, dh), q.dtype),
        scratch_shapes=[
            pltpu.VMEM((nh, dh), q.dtype),
            pltpu.VMEM((nh, dh), jnp.float32),
            pltpu.VMEM((nh, dh), jnp.float32),
            pltpu.VMEM((nh, dh), q.dtype),
            pltpu.VMEM((_SLOTS, dh, skv), k.dtype),
            pltpu.VMEM((_SLOTS, dh, skv), v.dtype),
            pltpu.SemaphoreType.DMA((_SLOTS,)),
            pltpu.SemaphoreType.DMA((_SLOTS,)),
            pltpu.SemaphoreType.DMA((3,)),
        ],
        compiler_params=pltpu.CompilerParams(
            vmem_limit_bytes=64 * 1024 * 1024,
            disable_bounds_checks=True,
            disable_semaphore_checks=True,
        ),
    )(q.reshape(nh, dh), kt, vt)
    return out.reshape(batch, heads, sq, dh)
```

```python
import jax
import jax.numpy as jnp
from jax import lax
import jax.experimental.pallas as pl
import jax.experimental.pallas.tpu as pltpu

_K, _V = 0, 1
_ROWS = 8
_HEADS = 4
_SEGMENTS = 6
_BACKLOG = 32
_DRAIN_BATCHES = 7
_LATE_ROWS = 16
_BOTH = slice(None)


def _interleave(*lists):
    out = []
    for i in range(max(map(len, lists))):
        out += [l[i] for l in lists if i < len(l)]
    return out


@jax.jit
def pallas_standalone__softmax_full_bidir__sampling_kernel(
    q: jax.Array,
    k: jax.Array,
    v: jax.Array,
):
    batch, heads, sq, dh = q.shape
    skv = k.shape[2]
    nh = batch * heads
    assert sq == 1
    scale = dh ** -0.5
    chunk = dh // 3
    windows = nh // _HEADS
    last_window = windows - 1
    last_slot = last_window % 2
    early = nh - _LATE_ROWS

    def kernel_function(q_hbm, k_hbm, v_hbm, o_hbm, q_in, q_f32, o_f32, o_out,
                        k_buf, v_buf, window_sem, drain_sem, io_sem):
        src, dst = (k_hbm, v_hbm), (k_buf, v_buf)

        def start(thread, op, window, seg, nseg, half, row, col, ncol, done):
            tile = (half, pl.ds(row, _ROWS), pl.ds(col, ncol))
            pltpu.make_async_copy(
                src[op].at[(pl.ds(window * _SEGMENTS + seg, nseg), *tile)],
                dst[op].at[(window % 2, pl.ds(seg, nseg), *tile)],
                done,
            ).start(priority=thread)

        def wait(ref, done):
            pltpu.make_async_copy(ref, ref, done).wait()

        def fetch_quarter(n):
            window, part = n // _HEADS, _HEADS - 1 - n % _HEADS
            rows, ncol = 2 * chunk // _HEADS, skv // 4
            for r in reversed(range(0, rows, _ROWS)):
                row = pl.multiple_of(part % 2 * rows + r, _ROWS)
                for col in reversed(range(0, skv, ncol)):
                    for seg in range(0, _SEGMENTS, 2):
                        for op in (_K, _V):
                            done = window_sem.at[window % 2 * 2 + op]
                            start(op, op, window, seg, 2, part // 2, row, col, ncol, done)

        def slab(op, slot, j):
            return jnp.concatenate(
                [dst[op][slot, (3 * j + i) // 2, (3 * j + i) % 2] for i in range(3)], axis=0
            )

        def softmax_weights(head, kt):
            q8 = jnp.broadcast_to(q_f32[pl.ds(head, 1), :], (8, dh)).astype(kt.dtype)
            s = jnp.dot(q8, kt, preferred_element_type=jnp.float32) * scale
            e = jnp.exp(s - jnp.max(s, axis=-1, keepdims=True))
            return e.astype(v_buf.dtype), 1.0 / jnp.sum(e, axis=-1, keepdims=True)

        def weighted_sum(e, inv_denom, vt):
            out = lax.dot_general(
                e, vt, (((1,), (1,)), ((), ())), preferred_element_type=jnp.float32
            )
            return (out * inv_denom)[0:1]

        parts = [(0, 3, _BOTH), (3, 1, _BOTH), (4, 1, 0), (4, 1, 1), (5, 1, _BOTH)]
        final_sem = drain_sem.at[2 * len(parts)]

        def part_copies(op, i):
            seg, nseg, half = parts[i]
            ncol = skv // 4 if half is _BOTH else skv // 2
            return [
                (op, last_window, s, 1, half, r, c, ncol, drain_sem.at[2 * i + op])
                for r in range(0, chunk, _ROWS)
                for c in range(0, skv, ncol)
                for s in range(seg, seg + nseg)
            ]

        def wait_part(op, i):
            seg, nseg, half = parts[i]
            wait(dst[op].at[last_slot, pl.ds(seg, nseg), half], drain_sem.at[2 * i + op])

        def head_copies(op, big, small):
            big = part_copies(op, big)
            return _interleave(big[0::2], part_copies(op, small), big[1::2])

        final = part_copies(_V, 3)
        landing_order = (
            _interleave(part_copies(_K, 0), part_copies(_V, 0))
            + _interleave(head_copies(_K, 1, 2), head_copies(_V, 1, 2))
            + head_copies(_K, 4, 3)
            + part_copies(_V, 4)
            + final[0::2]
            + [(*c[:-1], final_sem) for c in final[1::2]]
        )
        thread0 = landing_order[:_BACKLOG] + landing_order[_BACKLOG:-_BACKLOG:2]
        thread1 = landing_order[_BACKLOG + 1:-_BACKLOG:2] + landing_order[-_BACKLOG:]
        drain = _interleave([(0, *c) for c in thread0], [(1, *c) for c in thread1])
        size = len(drain) // (_DRAIN_BATCHES + 1)
        cuts = [0] + [size * (i + 2) for i in range(_DRAIN_BATCHES)]

        q_copy = pltpu.make_async_copy(q_hbm, q_in, io_sem.at[0])
        q_copy.start()

        def step(n, _):
            head = n - _HEADS

            @pl.when(n < nh - _HEADS)
            def _():
                fetch_quarter(n)

            for i in range(_DRAIN_BATCHES):
                @pl.when(n == nh - _HEADS + i)
                def _():
                    for c in drain[cuts[i]:cuts[i + 1]]:
                        start(*c)

            @pl.when(head == -1)
            def _():
                q_copy.wait()
                q_f32[...] = q_in[...].astype(jnp.float32)

            @pl.when(head == nh - _HEADS)
            def _():
                o_out[:early] = o_f32[:early].astype(o_out.dtype)
                for op in (_K, _V):
                    wait_part(op, 0)

            @pl.when(head == nh - 2)
            def _():
                for op in (_K, _V):
                    wait_part(op, 1)
                    wait_part(op, 2)

            @pl.when(head >= 0)
            def _():
                slot, j = head // _HEADS % 2, head % _HEADS

                @pl.when((j == 0) & (head < nh - _HEADS))
                def _():
                    for op in (_K, _V):
                        wait(dst[op].at[slot], window_sem.at[slot * 2 + op])

                e, inv_denom = softmax_weights(head, slab(_K, slot, j))
                o_f32[pl.ds(head, 1), :] = weighted_sum(e, inv_denom, slab(_V, slot, j))

        lax.fori_loop(0, nh + _HEADS - 1, step, None)

        wait_part(_K, 3)
        wait_part(_K, 4)
        e, inv_denom = softmax_weights(nh - 1, slab(_K, last_slot, _HEADS - 1))
        wait_part(_V, 4)
        v_hi = v_buf[last_slot, 5].reshape(2 * chunk, skv)
        o_f32[nh - 1:, chunk:] = weighted_sum(e, inv_denom, v_hi)
        mid = skv // 2
        wait(v_buf.at[last_slot, 4, 1, :, :mid], drain_sem.at[2 * 3 + _V])
        early_copy = pltpu.make_async_copy(
            o_out.at[pl.ds(0, early)], o_hbm.at[pl.ds(0, early)], io_sem.at[1]
        )
        early_copy.start()
        o_f32[nh - 1:, :chunk] = weighted_sum(
            e[:, :mid], inv_denom, v_buf[last_slot, 4, 1, :, :mid]
        )
        wait(v_buf.at[last_slot, 4, 1, :, mid:], final_sem)
        o_f32[nh - 1:, :chunk] += weighted_sum(
            e[:, mid:], inv_denom, v_buf[last_slot, 4, 1, :, mid:]
        )
        o_out[early:] = o_f32[early:].astype(o_out.dtype)
        late_copy = pltpu.make_async_copy(
            o_out.at[pl.ds(early, _LATE_ROWS)], o_hbm.at[pl.ds(early, _LATE_ROWS)],
            io_sem.at[2],
        )
        late_copy.start()
        early_copy.wait()
        late_copy.wait()

    def segments(x):
        return jnp.swapaxes(x, 2, 3).reshape(windows * _SEGMENTS, 2, chunk, skv)

    hbm = pl.BlockSpec(memory_space=pl.ANY)
    out = pl.pallas_call(
        kernel_function,
        in_specs=[hbm, hbm, hbm],
        out_specs=hbm,
        out_shape=jax.ShapeDtypeStruct((nh, dh), q.dtype),
        scratch_shapes=[
            pltpu.VMEM((nh, dh), q.dtype),
            pltpu.VMEM((nh, dh), jnp.float32),
            pltpu.VMEM((nh, dh), jnp.float32),
            pltpu.VMEM((nh, dh), q.dtype),
            pltpu.VMEM((2, _SEGMENTS, 2, chunk, skv), k.dtype),
            pltpu.VMEM((2, _SEGMENTS, 2, chunk, skv), v.dtype),
            pltpu.SemaphoreType.DMA((4,)),
            pltpu.SemaphoreType.DMA((11,)),
            pltpu.SemaphoreType.DMA((3,)),
        ],
        compiler_params=pltpu.CompilerParams(
            vmem_limit_bytes=64 * 1024 * 1024,
            disable_bounds_checks=True,
            disable_semaphore_checks=True,
        ),
    )(q.reshape(nh, dh), segments(k), segments(v))
    return out.reshape(batch, heads, sq, dh)
```

```python
import jax
import jax.numpy as jnp
from jax import lax
import jax.experimental.pallas as pl
import jax.experimental.pallas.tpu as pltpu

_K, _V = 0, 1
_ROWS = 8
_HEADS = 8
_SEGMENTS = 12
_FETCH_STEPS = _HEADS // 2
_BACKLOG = 26
_IN_FLIGHT = 110
_LATE_ROWS = 16


def _start_order(copies):
    out, served = [], 0
    for copy in copies:
        served += copy[0]
        out.append((served if copy[0] else served + _BACKLOG + 0.5, copy))
    return out, served


def _step_copies(rows, cols):
    timed, total = _start_order([
        (thread, seg + first, count, row, col)
        for row in rows
        for col in cols
        for seg in range(0, _SEGMENTS, 3)
        for thread, first, count in ((0, 0, 1), (1, 1, 2))
    ])
    wrapped = [(t - total, True, *c) if t > total + 0.5 else (t, False, *c) for t, c in timed]
    return [c[1:] for c in sorted(wrapped)]


def _drain_copies(rows, cols):
    final = 3 * (_HEADS - 1)
    paced = []
    for chunk in range(3 * _HEADS):
        period = (_HEADS - chunk // 3) ** -2
        parts = [(cols, period)]
        if chunk == final:
            parts = [(cols[:len(cols) // 2], 3 * period), (cols[len(cols) // 2:], 8 * period)]
        for part_cols, due in parts:
            pieces = [(chunk, row, col) for row in rows for col in part_cols]
            paced += [((i + 0.5) / len(pieces) * due, chunk % 2, p) for i, p in enumerate(pieces)]
    pieces = [p[-1] for p in sorted(paced)]
    timed, _ = _start_order([(min(i % 3, 1), *p) for i, p in enumerate(pieces)])
    copies = [c for _, c in sorted(timed)]
    ends = [
        min(len(pieces), max(i for i, p in enumerate(pieces) if p[0] // 3 == j) + _IN_FLIGHT)
        for j in range(_HEADS - 1)
    ]
    lead_in = _FETCH_STEPS + 2
    ends = [ends[0] * i // lead_in for i in range(lead_in)] + ends[:-1] + [len(pieces)]
    return [copies[a:b] for a, b in zip(ends, ends[1:])]


@jax.jit
def pallas_standalone__softmax_full_bidir__sampling_kernel(
    q: jax.Array,
    k: jax.Array,
    v: jax.Array,
):
    batch, heads, sq, dh = q.shape
    skv = k.shape[2]
    nh = batch * heads
    assert sq == 1
    scale = dh ** -0.5
    chunk_rows = dh // 3
    step_rows = 2 * chunk_rows // _FETCH_STEPS
    ncol = skv // 4
    windows = nh // _HEADS
    last_k = (windows - 1) % 2 * 2
    last_v = last_k + 1
    final = 3 * (_HEADS - 1)
    early = nh - _LATE_ROWS
    cols = list(range(0, skv, ncol))
    step_copies = _step_copies(range(0, step_rows, _ROWS), cols)
    drain_copies = _drain_copies(range(0, chunk_rows, _ROWS), cols)

    def kernel_function(q_hbm, k_hbm, v_hbm, o_hbm, q_in, q_f32, o_f32, o_out,
                        last_e, last_inv, buf, window_sem, drain_sem, io_sem):
        def wait(ref, done):
            pltpu.make_async_copy(ref, ref, done).wait()

        def fetcher(n):
            window, part = n // _HEADS, n % _FETCH_STEPS
            rows = (part // 2, pl.ds(pl.multiple_of(part % 2 * step_rows, step_rows), step_rows))
            segments = pl.ds(window * _SEGMENTS, _SEGMENTS)

            def start(op, thread, seg, count, row, col):
                slot = window % 2 * 2 + op
                piece = (pl.ds(seg, count), pl.ds(row, _ROWS), pl.ds(col, ncol))
                pltpu.make_async_copy(
                    (k_hbm, v_hbm)[op].at[(segments, *rows)].at[piece],
                    buf.at[(slot, slice(None), *rows)].at[piece],
                    window_sem.at[slot],
                ).start(priority=thread)

            return start

        def start_drain(batch_index):
            for thread, chunk, row, col in drain_copies[batch_index]:
                piece = (chunk % 2, pl.ds(row, _ROWS), pl.ds(col, ncol))
                is_last = chunk == final and col >= skv // 2
                pltpu.make_async_copy(
                    v_hbm.at[((windows - 1) * _SEGMENTS + chunk // 2, *piece)],
                    buf.at[(last_v, chunk // 2, *piece)],
                    drain_sem.at[3 * _HEADS if is_last else chunk],
                ).start(priority=thread)

        def wait_chunk(chunk):
            wait(buf.at[last_v, chunk // 2, chunk % 2], drain_sem.at[chunk])

        def slab(slot, j):
            return jnp.concatenate(
                [buf[slot, (3 * j + i) // 2, (3 * j + i) % 2] for i in range(3)], axis=0
            )

        def softmax_weights(head, kt):
            q8 = jnp.broadcast_to(q_f32[pl.ds(head, 1), :], (8, dh)).astype(kt.dtype)
            s = jnp.dot(q8, kt, preferred_element_type=jnp.float32) * scale
            e = jnp.exp(s - jnp.max(s, axis=-1, keepdims=True))
            return e, 1.0 / jnp.sum(e, axis=-1, keepdims=True)

        def weighted_sum(e, inv_denom, vt):
            out = lax.dot_general(
                e.astype(vt.dtype), vt, (((1,), (1,)), ((), ())),
                preferred_element_type=jnp.float32,
            )
            return (out * inv_denom)[0:1]

        q_copy = pltpu.make_async_copy(q_hbm, q_in, io_sem.at[0])
        q_copy.start()

        def step(n, _):
            head = n - _HEADS
            first_drain = nh - _FETCH_STEPS
            previous = jnp.maximum(n - 1, 0)
            start, start_previous = fetcher(n), fetcher(previous)

            for op in (_K, _V):
                @pl.when((n < first_drain) & (n // _FETCH_STEPS % 2 == op))
                def _():
                    for delayed, *copy in step_copies:
                        if not delayed:
                            start(op, *copy)
                            continue
                        for previous_op in (_K, _V):
                            @pl.when((n > 0) & (previous // _FETCH_STEPS % 2 == previous_op))
                            def _():
                                start_previous(previous_op, *copy)

            for i in range(_FETCH_STEPS + _HEADS - 1):
                @pl.when(n == first_drain + i)
                def _():
                    if i == 0:
                        for delayed, *copy in step_copies:
                            if delayed:
                                start_previous(_K, *copy)
                    if i <= _FETCH_STEPS:
                        start_drain(i)
                    if i == _FETCH_STEPS:
                        wait(buf.at[last_k], window_sem.at[last_k])
                        o_out[:early] = o_f32[:early].astype(o_out.dtype)
                        e, inv_denom = softmax_weights(nh - 1, slab(last_k, _HEADS - 1))
                        last_e[...] = e
                        last_inv[...] = jnp.broadcast_to(inv_denom, last_inv.shape)
                    if i >= _FETCH_STEPS:
                        start_drain(i + 1)

            @pl.when(head == -1)
            def _():
                q_copy.wait()
                q_f32[...] = q_in[...].astype(jnp.float32)

            @pl.when(head >= 0)
            def _():
                slot, j = head // _HEADS % 2 * 2, head % _HEADS

                @pl.when((j == 0) & (head < nh - _HEADS))
                def _():
                    for op in (_K, _V):
                        wait(buf.at[slot + op], window_sem.at[slot + op])

                @pl.when(head >= nh - _HEADS)
                def _():
                    for i in range(3):
                        wait_chunk(3 * j + i)

                e, inv_denom = softmax_weights(head, slab(slot + _K, j))
                o_f32[pl.ds(head, 1), :] = weighted_sum(e, inv_denom, slab(slot + _V, j))

        lax.fori_loop(0, nh + _HEADS - 1, step, None)

        wait_chunk(final + 1)
        wait_chunk(final + 2)
        o_f32[nh - 1:, chunk_rows:] = weighted_sum(
            last_e[...], last_inv[:, :1], buf[last_v, _SEGMENTS - 1].reshape(2 * chunk_rows, skv)
        )
        early_copy = pltpu.make_async_copy(
            o_out.at[pl.ds(0, early)], o_hbm.at[pl.ds(0, early)], io_sem.at[1]
        )
        lo, hi = pl.ds(0, skv // 2), pl.ds(skv // 2, skv // 2)
        v_lo, v_hi = (buf.at[last_v, final // 2, final % 2, :, keys] for keys in (lo, hi))
        wait(v_lo, drain_sem.at[final])
        early_copy.start()
        o_f32[nh - 1:, :chunk_rows] = weighted_sum(
            last_e[:, lo], last_inv[:, :chunk_rows], v_lo[...]
        )
        wait(v_hi, drain_sem.at[3 * _HEADS])
        o_f32[nh - 1:, :chunk_rows] += weighted_sum(
            last_e[:, hi], last_inv[:, :chunk_rows], v_hi[...]
        )
        o_out[early:] = o_f32[early:].astype(o_out.dtype)
        late_copy = pltpu.make_async_copy(
            o_out.at[pl.ds(early, _LATE_ROWS)], o_hbm.at[pl.ds(early, _LATE_ROWS)],
            io_sem.at[2],
        )
        late_copy.start()
        early_copy.wait()
        late_copy.wait()

    def as_segments(x):
        return jnp.swapaxes(x, 2, 3).reshape(windows * _SEGMENTS, 2, chunk_rows, skv)

    hbm = pl.BlockSpec(memory_space=pl.ANY)
    out = pl.pallas_call(
        kernel_function,
        in_specs=[hbm, hbm, hbm],
        out_specs=hbm,
        out_shape=jax.ShapeDtypeStruct((nh, dh), q.dtype),
        scratch_shapes=[
            pltpu.VMEM((nh, dh), q.dtype),
            pltpu.VMEM((nh, dh), jnp.float32),
            pltpu.VMEM((nh, dh), jnp.float32),
            pltpu.VMEM((nh, dh), q.dtype),
            pltpu.VMEM((8, skv), jnp.float32),
            pltpu.VMEM((8, 128), jnp.float32),
            pltpu.VMEM((4, _SEGMENTS, 2, chunk_rows, skv), k.dtype),
            pltpu.SemaphoreType.DMA((4,)),
            pltpu.SemaphoreType.DMA((3 * _HEADS + 1,)),
            pltpu.SemaphoreType.DMA((3,)),
        ],
        compiler_params=pltpu.CompilerParams(
            vmem_limit_bytes=64 * 1024 * 1024,
            disable_bounds_checks=True,
            disable_semaphore_checks=True,
        ),
    )(q.reshape(nh, dh), as_segments(k), as_segments(v))
    return out.reshape(batch, heads, sq, dh)
```

```python
import jax
import jax.numpy as jnp
from jax import lax
import jax.experimental.pallas as pl
import jax.experimental.pallas.tpu as pltpu

_ROWS, _LANES = 8, 128
_HEADS = 8
_SEGMENTS = 12
_OFFSET = 2
_BACKLOG = 25
_K_LAG, _K_SLOTS = _HEADS + 1, 3
_V_LAG, _V_SLOTS = 2, 3
_LATE_ROWS = 16


def _step_copies(rows, cols):
    timed, served = [], 0
    for row in rows:
        for col in cols:
            for seg in range(0, _SEGMENTS, 3):
                served += 1
                timed.append((served, 1, seg, 2, row, col))
                timed.append((served + _BACKLOG + 0.5, 0, seg + 2, 1, row, col))
    wrapped = [
        (t - served, True, *copy) if t > served + 0.5 else (t, False, *copy)
        for t, *copy in timed
    ]
    return [copy[1:] for copy in sorted(wrapped)]


@jax.jit
def pallas_standalone__softmax_full_bidir__sampling_kernel(
    q: jax.Array,
    k: jax.Array,
    v: jax.Array,
):
    batch, heads, sq, dh = q.shape
    skv = k.shape[2]
    nh = batch * heads
    chunk_rows = dh // 3
    step_rows = 2 * chunk_rows // _HEADS
    assert sq == 1 and step_rows == 2 * _ROWS and nh % _HEADS == 0
    scale = dh ** -0.5
    ncol = skv // 4
    last_col = skv - ncol
    step_copies = _step_copies(range(0, step_rows, _ROWS), range(0, skv, ncol))

    def kernel_function(q_hbm, k_hbm, v_hbm, o_hbm, q_in, q_f32, weights, inv_denoms,
                        partial, o_f32, o_out, k_buf, v_buf, k_sem, v_sem, io_sem):
        def wait(ref, done):
            pltpu.make_async_copy(ref, ref, done).wait()

        def locate(n):
            window = pl.multiple_of(nh - _HEADS - n // _HEADS * _HEADS, _HEADS)
            part = n % _HEADS
            row = pl.multiple_of(part % (_HEADS // 2) * step_rows, step_rows)
            return window, part // (_HEADS // 2), row

        def fetcher(n, is_v):
            window, half, row0 = locate(n)
            rows = (half, pl.ds(row0, step_rows))
            pairs = [(window + _OFFSET + 2 * i) % nh // 2 * 3 for i in range(_HEADS // 2)]
            if is_v:
                slot = n % _V_SLOTS
                src, dst = v_hbm, v_buf.at[slot]
                sems = [v_sem.at[jnp.where(n == nh - 1, _V_SLOTS + i, slot)] for i in range(3)]
            else:
                slot = n // _HEADS % _K_SLOTS
                src, dst = k_hbm, k_buf.at[(slot, slice(None), *rows)]
                sems = [k_sem.at[slot]] * 3

            def start(thread, seg, count, row, col):
                tile = (pl.ds(row, _ROWS), pl.ds(col, ncol))
                segments = src.at[(pl.ds(pairs[seg // 3] + seg % 3, count), *rows)]
                pltpu.make_async_copy(
                    segments.at[(slice(None), *tile)],
                    dst.at[(pl.ds(seg, count), *tile)],
                    sems[0 if row == 0 else 1 if col < last_col else 2],
                ).start(priority=thread)

            return start

        def softmax_weights(n):
            window, _, _ = locate(n)
            slot, j = n // _HEADS % _K_SLOTS, n % _HEADS

            @pl.when(j == 0)
            def _():
                wait(k_buf.at[slot], k_sem.at[slot])

            kt = jnp.concatenate(
                [k_buf[slot, (3 * j + i) // 2, (3 * j + i) % 2] for i in range(3)], axis=0
            )
            q_row = q_f32[pl.ds((window + j + _OFFSET) % nh, 1), :]
            q8 = jnp.broadcast_to(q_row, (8, dh)).astype(kt.dtype)
            s = jnp.dot(q8, kt, preferred_element_type=jnp.float32) * scale
            e = jnp.exp(s - jnp.max(s, axis=-1, keepdims=True))
            inv_denom = 1.0 / jnp.sum(e, axis=-1, keepdims=True)
            weights[pl.ds(window + j, 1), :] = e[:1]
            inv_denoms[pl.ds(window + j, 1), :] = jnp.broadcast_to(inv_denom[:1], (1, _LANES))

        def weighted_sums(window, keys, vt):
            e = weights[pl.ds(window, _HEADS), keys].astype(vt.dtype)
            return lax.dot_general(
                e, vt.reshape(-1, vt.shape[-1]), (((1,), (1,)), ((), ())),
                preferred_element_type=jnp.float32,
            )

        def store_own_rows(window, half, row0, sums):
            rows = sums.shape[1] // _SEGMENTS
            window = pl.ds(window, _HEADS)
            sums = jnp.pad(sums, ((0, 0), (0, -sums.shape[1] % _LANES)))
            sums = [sums[:, i:i + _LANES] * inv_denoms[window, :]
                    for i in range(0, sums.shape[1], _LANES)]
            head = lax.broadcasted_iota(jnp.int32, (_HEADS, 2 * _LANES), 0)
            lane = lax.broadcasted_iota(jnp.int32, (_HEADS, 2 * _LANES), 1)
            out = o_f32[window, :]
            for seg in range(_SEGMENTS):
                chunk = 2 * seg + half
                to = chunk % 3 * chunk_rows + row0
                tile, at = divmod(seg * rows, _LANES)
                moved = pltpu.roll(sums[tile], (to + _LANES - at) % _LANES, 1)
                own = (head == chunk // 3) & (lane >= to) & (lane < to + rows)
                out = jnp.where(own, jnp.concatenate([moved, moved], axis=1), out)
            o_f32[window, :] = out

        q_copy = pltpu.make_async_copy(q_hbm, q_in, io_sem.at[0])
        q_copy.start()

        def step(n, _):
            def fetchers(m):
                return [
                    ((m >= is_v * nh) & (m < is_v * nh + nh),
                     fetcher(jnp.clip(m - is_v * nh, 0, nh - 1), is_v))
                    for is_v in (0, 1)
                ]

            previous = fetchers(n - 1)
            for active, start in fetchers(n):
                @pl.when(active)
                def _():
                    for delayed, *copy in step_copies:
                        if not delayed:
                            start(*copy)
                            continue
                        for was_active, start_previous in previous:
                            @pl.when(was_active)
                            def _():
                                start_previous(*copy)

            @pl.when(n == 2 * nh)
            def _():
                for delayed, *copy in step_copies:
                    if delayed:
                        previous[1][1](*copy)

            @pl.when(n == _K_LAG - 1)
            def _():
                q_copy.wait()
                q_f32[...] = q_in[...].astype(jnp.float32)
                o_f32[...] = jnp.zeros_like(o_f32)

            @pl.when((n >= _K_LAG) & (n < nh + _K_LAG))
            def _():
                softmax_weights(n - _K_LAG)

            @pl.when(n >= nh + _V_LAG)
            def _():
                m = n - nh - _V_LAG
                window, half, row0 = locate(m)
                slot = m % _V_SLOTS
                wait(v_buf.at[slot], v_sem.at[slot])
                sums = weighted_sums(window, slice(None), v_buf[slot])
                store_own_rows(window, half, row0, sums)

            @pl.when(n == 2 * nh - 2)
            def _():
                done = o_f32[_LATE_ROWS - _OFFSET:nh - _OFFSET, :dh]
                o_out[_LATE_ROWS:] = done.astype(o_out.dtype)

        lax.fori_loop(0, 2 * nh + _V_LAG - 1, step, None)

        early, late = pl.ds(_LATE_ROWS, nh - _LATE_ROWS), pl.ds(0, _LATE_ROWS)
        early_copy = pltpu.make_async_copy(o_out.at[early], o_hbm.at[early], io_sem.at[1])
        late_copy = pltpu.make_async_copy(o_out.at[late], o_hbm.at[late], io_sem.at[2])
        last = v_buf.at[(nh - 1) % _V_SLOTS]
        lo, hi = slice(0, last_col), slice(last_col, skv)
        pieces = last.at[:, :_ROWS], last.at[:, _ROWS:, lo], last.at[:, _ROWS:, hi]

        wait(pieces[0], v_sem.at[_V_SLOTS])
        sums = weighted_sums(0, slice(None), pieces[0][...])
        store_own_rows(0, 1, chunk_rows - step_rows, sums)
        wait(pieces[1], v_sem.at[_V_SLOTS + 1])
        early_copy.start()
        partial[...] = weighted_sums(0, lo, pieces[1][...])
        wait(pieces[2], v_sem.at[_V_SLOTS + 2])
        sums = weighted_sums(0, hi, pieces[2][...]) + partial[...]
        store_own_rows(0, 1, chunk_rows - _ROWS, sums)
        done = jnp.concatenate(
            [o_f32[nh - _OFFSET:, :dh], o_f32[:_LATE_ROWS - _OFFSET, :dh]], axis=0
        )
        o_out[:_LATE_ROWS] = done.astype(o_out.dtype)
        late_copy.start()
        early_copy.wait()
        late_copy.wait()

    def as_segments(x):
        return jnp.swapaxes(x, 2, 3).reshape(-1, 2, chunk_rows, skv)

    hbm = pl.BlockSpec(memory_space=pl.ANY)
    out = pl.pallas_call(
        kernel_function,
        in_specs=[hbm, hbm, hbm],
        out_specs=hbm,
        out_shape=jax.ShapeDtypeStruct((nh, dh), q.dtype),
        scratch_shapes=[
            pltpu.VMEM((nh, dh), q.dtype),
            pltpu.VMEM((nh, dh), jnp.float32),
            pltpu.VMEM((nh, skv), jnp.float32),
            pltpu.VMEM((nh, _LANES), jnp.float32),
            pltpu.VMEM((_HEADS, _SEGMENTS * _ROWS), jnp.float32),
            pltpu.VMEM((nh, 2 * _LANES), jnp.float32),
            pltpu.VMEM((nh, dh), q.dtype),
            pltpu.VMEM((_K_SLOTS, _SEGMENTS, 2, chunk_rows, skv), k.dtype),
            pltpu.VMEM((_V_SLOTS, _SEGMENTS, step_rows, skv), v.dtype),
            pltpu.SemaphoreType.DMA((_K_SLOTS,)),
            pltpu.SemaphoreType.DMA((_V_SLOTS + 3,)),
            pltpu.SemaphoreType.DMA((3,)),
        ],
        compiler_params=pltpu.CompilerParams(
            vmem_limit_bytes=64 * 1024 * 1024,
            disable_bounds_checks=True,
            disable_semaphore_checks=True,
        ),
    )(q.reshape(nh, dh), as_segments(k), as_segments(v))
    return out.reshape(batch, heads, sq, dh)
```
